```python
import os as _os
_os.environ.setdefault("JAX_PLATFORMS", "cpu")
import jax
import jax.numpy as jnp

def _softmax(x, axis=-1):
    return jax.nn.softmax(x, axis=axis)
def _gelu(x):
    return jax.nn.gelu(x, approximate=True)
def _silu(x):
    return jax.nn.silu(x)
def _sigmoid(x):
    return jax.nn.sigmoid(x)
def _layernorm(x, axis=-1, eps=1e-5):
    m = jnp.mean(x, axis=axis, keepdims=True)
    v = jnp.var(x, axis=axis, keepdims=True)
    return (x - m) / jnp.sqrt(v + eps)
def _scatter_add(tgt, idx, src, axis=0):
    return tgt.at[idx].add(src)
def _segment_sum(src, seg, n):
    return jax.ops.segment_sum(src, seg, n)
class _Rng:
    def __init__(self, key):
        self._k = key
    def _next(self):
        self._k, sub = jax.random.split(self._k)
        return sub
    def normal(self, shape):
        return jax.random.normal(self._next(), shape, dtype=jnp.bfloat16)
    def randint(self, lo, hi, shape):
        return jax.random.randint(self._next(), shape, lo, hi, dtype=jnp.int32)
    def uniform(self, shape, lo=0.0, hi=1.0):
        return jax.random.uniform(self._next(), shape, jnp.bfloat16, lo, hi)
    def permutation(self, n):
        return jax.random.permutation(self._next(), n)


kernel_name = 'sequential_preLN__mha_block__mixer_token_mlp__prompt'

def setup_inputs():
    _rng = _Rng(jax.random.key(int.from_bytes(__import__("os").urandom(4), "little")))
    _w = (lambda a: (lambda t: t.astype(jnp.bfloat16) if jnp.issubdtype(t.dtype, jnp.floating) else t)(jnp.asarray(a)))
    def _A_setup():
        B, S, D, H = 1, 2048, 448, 16
        return {
            "x": _w((lambda *s: _rng.normal(s) * 0.05)(B, S, D)),
            "wqkv": _w((lambda *s: _rng.normal(s) * 0.05)(D, 3 * D)),
            "wo": _w((lambda *s: _rng.normal(s) * 0.05)(D, D)),
        }
    _A_in = _A_setup()

    def _B_setup():
        B, S, D, F = 1, 2048, 448, 1792
        return {
            "x": _w((lambda *s: _rng.normal(s) * 0.05)(B, S, D)),
            "w1": _w((lambda *s: _rng.normal(s) * 0.2)(S, F) * (S ** -0.5)),
            "b1": _w((lambda *s: _rng.normal(s) * 0.2)(F) * 0.02),
            "w2": _w((lambda *s: _rng.normal(s) * 0.2)(F, S) * (F ** -0.5)),
            "b2": _w((lambda *s: _rng.normal(s) * 0.05)(S) * 0.02),
        }
    _B_in = _B_setup()

    return {
        "A_x": _A_in["x"],
        "A_wqkv": _A_in["wqkv"],
        "A_wo": _A_in["wo"],
        "B_x": _B_in["x"],
        "B_w1": _B_in["w1"],
        "B_b1": _B_in["b1"],
        "B_w2": _B_in["w2"],
        "B_b2": _B_in["b2"],
    }

def reference(A_x, A_wqkv, A_wo, B_x, B_w1, B_b1, B_w2, B_b2):
    def _A_ref(x, wqkv, wo):
        B, S, D = x.shape
        H = 16
        Dh = D // H
        qkv = (lambda x, *d: x.transpose(*d))((x @ wqkv).reshape(B, S, 3, H, Dh), 2, 0, 3, 1, 4)
        q, k, v = qkv[0], qkv[1], qkv[2]
        scores = jnp.einsum("bhqd,bhkd->bhqk", q, k) * (Dh ** -0.5)
        p = _softmax(scores, axis=-1)
        o = jnp.einsum("bhqk,bhkd->bhqd", p, v)
        return (lambda x, *d: x.transpose(*d))(o, 0, 2, 1, 3).reshape(B, S, D) @ wo

    def _B_ref(x, w1, b1, w2, b2):
        B, S, D = x.shape
        h = _layernorm(x, axis=-1)
        u = jnp.einsum("bsd,sf->bdf", h, w1) + b1
        u = _gelu(u)
        y = jnp.einsum("bdf,fs->bds", u, w2) + b2
        return (lambda x, *d: x.transpose(*d))(y, 0, 2, 1)

    x = A_x
    h = x + _A_ref(_layernorm(x, axis=-1), A_wqkv, A_wo)
    h2 = h + _B_ref(_layernorm(h, axis=-1), B_w1, B_b1, B_w2, B_b2)
    return h2
```

```python
import math
import jax, jax.numpy as jnp
from jax.experimental import pallas as pl
from jax.experimental.pallas import tpu as pltpu

S, D, H, DH, DP, F = 2048, 448, 16, 28, 32, 1792
DPAD = H * DP
QB = 512
NQB = S // QB
CK = 128
NC = S // CK
UPI = 4
LAG = 1
FC = 256
TC = 256
f32, bf16 = jnp.float32, jnp.bfloat16
QSCALE = (DH ** -0.5) * math.log2(math.e)
EPS = 1e-5


def _gelu(x):
    c = math.sqrt(2.0 / math.pi)
    return 0.5 * x * (1.0 + jnp.tanh(c * (x + 0.044715 * (x * x * x))))


def _ln_cols(x):
    mu = jnp.mean(x, axis=0, keepdims=True)
    xc = x - mu
    var = jnp.mean(xc * xc, axis=0, keepdims=True)
    return xc * jax.lax.rsqrt(var + EPS)


def kernel(xT_hbm, wqkv_hbm, wo_hbm, b1_ref, b2_ref, w1_hbm, w2_hbm, out_hbm,
           z_ref, sems, xT_v, wqkv_v, wo_v, w1_v, w2_v, wt_f, wTp, woTp,
           k_s, qT_s, vT_s, oT_s, sA, sB, mA, mB, qmA, qmB, hT_s, ln2T_s, g_s, out_v):
    cp_wqkv = pltpu.make_async_copy(wqkv_hbm, wqkv_v, sems.at[0])
    cp_wqkv.start()
    cp_x = [pltpu.make_async_copy(xT_hbm.at[:, c * QB:(c + 1) * QB], xT_v.at[:, c * QB:(c + 1) * QB], sems.at[1 + c])
            for c in range(NQB)]
    for cp in cp_x:
        cp.start()
    cp_wo = pltpu.make_async_copy(wo_hbm, wo_v, sems.at[5]); cp_wo.start()
    cp1 = pltpu.make_async_copy(w1_hbm, w1_v, sems.at[6])
    cp2 = pltpu.make_async_copy(w2_hbm, w2_v, sems.at[7])

    z_ref[0] = 0
    z_ref[1] = 0
    sB_st = sB.at[z_ref[0]]
    sB_ld = sB.at[z_ref[1]]
    qmA[...] = jnp.zeros(qmA.shape, bf16)
    qmB[...] = jnp.zeros(qmB.shape, bf16)

    cp_wqkv.wait()
    for c in range(11):
        lo = c * 128
        hi = min(lo + 128, 3 * D)
        wt_f[lo:hi, :] = wqkv_v[:, lo:hi].astype(f32).T
    zpad = jnp.zeros((DP - DH, D), f32)
    for part, src in enumerate((1, 0, 2)):
        for h in range(H):
            r = src * D + h * DH
            blk = jnp.concatenate([wt_f[r:r + DH, :], zpad], axis=0).astype(bf16)
            wTp[part * DPAD + h * DP: part * DPAD + (h + 1) * DP, :] = blk

    for c in range(NQB):
        cp_x[c].wait()
        if c == NQB - 1:
            cp1.start()
            cp2.start()
        cs = slice(c * QB, (c + 1) * QB)
        ln = _ln_cols(xT_v[:, cs].astype(f32)).astype(bf16)
        kT = jnp.dot(wTp[0:DPAD, :], ln, preferred_element_type=f32)
        k = kT.T.astype(bf16)
        for g in range(4):
            k_s[g, cs, :] = k[:, g * 128:(g + 1) * 128]
        q = jnp.dot(wTp[DPAD:2 * DPAD, :], ln, preferred_element_type=f32)
        qT_s[c] = (q * QSCALE).astype(bf16)
        v = jnp.dot(wTp[2 * DPAD:, :], ln, preferred_element_type=f32)
        row = jax.lax.broadcasted_iota(jnp.int32, v.shape, 0)
        v = jnp.where(row % DP == DH, 1.0, v).astype(bf16)
        for h in range(H):
            vT_s[h, :, cs] = v[h * DP:(h + 1) * DP]

    cp_wo.wait()
    wt_f[0:D, :] = wo_v[...].astype(f32)
    for h in range(H):
        wt_f[D + h * DP: D + (h + 1) * DP, :] = jnp.concatenate([wt_f[h * DH:(h + 1) * DH, :], zpad], axis=0)
    for g in range(4):
        woTp[:, g * 128:(g + 1) * 128] = wt_f[D + g * 128: D + (g + 1) * 128, :].T.astype(bf16)

    NU = H * NQB

    def prep_q(u, qm_ref):
        h = u // NQB
        qb = u % NQB
        j = h % 4
        blk = qT_s[qb, pl.ds(pl.multiple_of(h * DP, DP), DP), :]
        qm_ref[j, pl.ds(pl.multiple_of(j * DP, DP), DP), :] = blk

    def qk_chunk(u, c, qm_ref, s_ref, mrun):
        h = u // NQB
        g = h // 4
        j = h % 4
        kc = k_s[g, c * CK:(c + 1) * CK, :]
        s = jnp.dot(kc, qm_ref[j], preferred_element_type=f32)
        s_ref[c * CK:(c + 1) * CK, :] = s
        mc = jnp.max(s.reshape(CK // 8, 8, QB), axis=0)
        return mc if mrun is None else jnp.maximum(mrun, mc)

    def pv_chunk(u, c, s_ref, m, acc):
        h = u // NQB
        p = jnp.exp2(s_ref[c * CK:(c + 1) * CK, :] - m).astype(bf16)
        o = jnp.dot(vT_s[h, :, c * CK:(c + 1) * CK], p, preferred_element_type=f32)
        return o if acc is None else acc + o

    def finalize(u, acc):
        h = u // NQB
        qb = u % NQB
        l = acc[DH:DH + 1, :]
        oT_s[qb, pl.ds(pl.multiple_of(h * DP, DP), DP), :] = (acc * pl.reciprocal(l, approx=False)).astype(bf16)

    def half(u_cur, u_next, s_cur, m_cur, s_next, m_next, qm_next, qm_next2, u_next2, lag):
        m = m_cur[...]
        mrun = None
        acc = None
        prep_q(u_next2, qm_next2)
        for t in range(NC + lag):
            if t < NC:
                mrun = qk_chunk(u_next, t, qm_next, s_next, mrun)
            if t >= lag:
                acc = pv_chunk(u_cur, t - lag, s_cur, m, acc)
        m_next[...] = jnp.max(mrun, axis=0, keepdims=True)
        finalize(u_cur, acc)

    prep_q(0, qmA)
    prep_q(1, qmB)
    mrun = None
    for c in range(NC):
        mrun = qk_chunk(0, c, qmA, sA, mrun)
    mA[...] = jnp.max(mrun, axis=0, keepdims=True)

    def body(i, carry):
        for k in range(UPI // 2):
            u = UPI * i + 2 * k
            c1 = jnp.minimum(u + 1, NU - 1); c2 = jnp.minimum(u + 2, NU - 1); c3 = jnp.minimum(u + 3, NU - 1)
            half(u, c1, sA, mA, sB_st, mB, qmB, qmA, c2, LAG)
            half(u + 1, c2, sB_ld, mB, sA, mA, qmA, qmB, c3, LAG)
        return carry
    jax.lax.fori_loop(0, NU // UPI, body, 0)

    for c in range(NQB):
        cs = slice(c * QB, (c + 1) * QB)
        a = jnp.dot(woTp[...], oT_s[c], preferred_element_type=f32)
        hT = xT_v[:, cs].astype(f32) + a
        hT_s[:, cs] = hT
        ln2T_s[:, cs] = _ln_cols(hT).astype(bf16)

    b1 = b1_ref[...].astype(f32)
    b2 = b2_ref[...].astype(f32)
    cp1.wait()
    for c in range(F // FC):
        u = jnp.dot(ln2T_s[...], w1_v[:, c * FC:(c + 1) * FC], preferred_element_type=f32)
        n = FC // 128
        bias = jnp.concatenate([b1[c * n + t: c * n + t + 1, :] for t in range(n)], axis=1)
        g_s[:, c * FC:(c + 1) * FC] = _gelu(u + bias).astype(bf16)
    cp2.wait()
    cps = []
    for c in range(S // TC):
        cs = slice(c * TC, (c + 1) * TC)
        y = jnp.dot(g_s[...], w2_v[:, cs], preferred_element_type=f32)
        n = TC // 128
        bias = jnp.concatenate([b2[c * n + t: c * n + t + 1, :] for t in range(n)], axis=1)
        out_v[:, cs] = (y + bias + hT_s[:, cs]).astype(bf16)
        cp = pltpu.make_async_copy(out_v.at[:, cs], out_hbm.at[:, cs], sems.at[8 + c])
        cp.start()
        cps.append(cp)
    for cp in cps:
        cp.wait()


@jax.jit
def pallas_sequential_preLN__mha_block__mixer_token_mlp__prompt_kernel(A_x, A_wqkv, A_wo, B_x, B_w1, B_b1, B_w2, B_b2):
    hb = lambda a: pltpu.with_memory_space_constraint(a, pltpu.HBM)
    xT = A_x.reshape(S, D).T
    b1 = B_b1.reshape(F // 128, 128)
    b2 = B_b2.reshape(S // 128, 128)
    vm = pl.BlockSpec(memory_space=pltpu.VMEM)
    hbm = pl.BlockSpec(memory_space=pl.ANY)
    outT = pl.pallas_call(
        kernel,
        out_shape=jax.ShapeDtypeStruct((D, S), bf16),
        in_specs=[hbm, hbm, hbm, vm, vm, hbm, hbm],
        out_specs=hbm,
        scratch_shapes=[
            pltpu.SMEM((2,), jnp.int32),
            pltpu.SemaphoreType.DMA((8 + S // TC,)),
            pltpu.VMEM((D, S), bf16),
            pltpu.VMEM((D, 3 * D), bf16),
            pltpu.VMEM((D, D), bf16),
            pltpu.VMEM((S, F), bf16), pltpu.VMEM((F, S), bf16),
            pltpu.VMEM((3 * D, D), f32),
            pltpu.VMEM((3 * DPAD, D), bf16),
            pltpu.VMEM((D, DPAD), bf16),
            pltpu.VMEM((4, S, 128), bf16),
            pltpu.VMEM((NQB, DPAD, QB), bf16),
            pltpu.VMEM((H, DP, S), bf16),
            pltpu.VMEM((NQB, DPAD, QB), bf16),
            pltpu.VMEM((S, QB), f32), pltpu.VMEM((1, S, QB), f32),
            pltpu.VMEM((1, QB), f32), pltpu.VMEM((1, QB), f32),
            pltpu.VMEM((4, 128, QB), bf16), pltpu.VMEM((4, 128, QB), bf16),
            pltpu.VMEM((D, S), f32),
            pltpu.VMEM((D, S), bf16),
            pltpu.VMEM((D, F), bf16),
            pltpu.VMEM((D, S), bf16),
        ],
        compiler_params=pltpu.CompilerParams(vmem_limit_bytes=100 * 1024 * 1024),
    )(hb(xT), hb(A_wqkv), hb(A_wo), b1, b2, hb(B_w1), hb(B_w2))
    return outT.T.reshape(1, S, D)
```

```python
import math
import jax, jax.numpy as jnp
from jax.experimental import pallas as pl
from jax.experimental.pallas import tpu as pltpu

S, D, H, DH, DP, F = 2048, 448, 16, 28, 32, 1792
DPAD = H * DP
QB = 512
NQB = S // QB
NU = H * NQB
NT = S // 128
HD = D // 2
CK = 128
NC = S // CK
UPI = 8
LAG = 1
FC = 256
f32, bf16 = jnp.float32, jnp.bfloat16
QSCALE = (DH ** -0.5) * math.log2(math.e)
EPS = 1e-5


def _gelu(x):
    c = math.sqrt(2.0 / math.pi)
    return 0.5 * x * (1.0 + jnp.tanh(c * (x + 0.044715 * (x * x * x))))


def _colsum(x):
    n = x.shape[1]
    y = jnp.sum(x.reshape(8, 56, n), axis=0)
    y = jnp.sum(y.reshape(7, 8, n), axis=0)
    return jnp.sum(y, axis=0, keepdims=True)


def _ln_cols(x):
    mu = _colsum(x) * (1.0 / D)
    xc = x - mu
    var = _colsum(xc * xc) * (1.0 / D)
    return xc * jax.lax.rsqrt(var + EPS)


def _interleave(main, side):
    n, m = len(main), len(side)
    j = 0
    for i, f in enumerate(main):
        f()
        while j < m and (j + 1) * n <= (i + 1) * m:
            side[j]()
            j += 1
    while j < m:
        side[j]()
        j += 1


def kernel(xT_hbm, wqkv_hbm, wo_hbm, b1_ref, b2_ref, w1_hbm, w2_hbm, out_hbm,
           z_ref, sems, xT_v, wqkv_v, wo_v, w1_v, w2_v, wt_f, wT, woTp, ln1_s,
           k_s, qT_s, vT_s, oT_s, sA, sB, mA, mB, hT_s, ln2T_s, g_s, out_v):
    def xcopy(lo, hi, sem):
        return pltpu.make_async_copy(xT_hbm.at[:, lo:hi], xT_v.at[:, lo:hi], sems.at[sem])
    WQ = 512
    cp_x0 = xcopy(0, QB, 0)
    cp_wq = pltpu.make_async_copy(wqkv_hbm.at[:, 0:WQ], wqkv_v.at[:, 0:WQ], sems.at[1])
    cp_x1 = xcopy(QB, 2 * QB, 2)
    cp_x23 = xcopy(2 * QB, S, 3)
    cp_wkv = pltpu.make_async_copy(wqkv_hbm.at[:, WQ:], wqkv_v.at[:, WQ:], sems.at[4])
    cp_wo = pltpu.make_async_copy(wo_hbm, wo_v, sems.at[5])
    cp1 = pltpu.make_async_copy(w1_hbm, w1_v, sems.at[6])
    cp2 = pltpu.make_async_copy(w2_hbm, w2_v, sems.at[7])
    cp_x0.start()
    cp_wq.start()

    def ts(t):
        return slice(t * 128, (t + 1) * 128)

    z_ref[0] = 0
    z_ref[1] = 0
    sB_st = sB.at[z_ref[0]]
    sB_ld = sB.at[z_ref[1]]
    zpad = jnp.zeros((DP - DH, D), f32)
    rz0 = pl.ds(pl.multiple_of(z_ref[0], 16), D)
    rz1 = pl.ds(pl.multiple_of(z_ref[1], 16), D)

    def ln_stats(x):
        p = x[0:1, :]
        d = x - p
        md = _colsum(d) * (1.0 / D)
        var = jnp.maximum(_colsum(d * d) * (1.0 / D) - md * md, 0.0)
        return p + md, jax.lax.rsqrt(var + EPS)

    def ln_apply(src_ref, t, dst_ref, mu, r):
        dst_ref[:, ts(t)] = ((src_ref[rz1, ts(t)].astype(f32) - mu) * r).astype(bf16)

    def wt_chunk(c):
        def f():
            lo = c * 128
            hi = min(lo + 128, 3 * D)
            wT[lo:hi, :] = wqkv_v[:, lo:hi].astype(f32).T.astype(bf16)
        return f

    def ln1(t):
        def f():
            mu, r = ln_stats(xT_v[:, ts(t)].astype(f32))
            ln_apply(xT_v, t, ln1_s, mu, r)
        return f

    def proj_q(t):
        def f():
            q = jnp.dot(wT[0:D, :], ln1_s[:, ts(t)], preferred_element_type=f32)
            q = (q * QSCALE).astype(bf16)
            qT_s[t // 4, 0, :, ts(t % 4)] = q[0:HD]
            qT_s[t // 4, 1, :, ts(t % 4)] = q[HD:]
        return f

    def proj_k(t):
        def f():
            kT = jnp.dot(wT[D:2 * D, :], ln1_s[:, ts(t)], preferred_element_type=f32)
            k = kT.T.astype(bf16)
            for h in range(H):
                k_s[h, ts(t), :] = k[:, h * DH:(h + 1) * DH]
        return f

    vtail = jnp.concatenate([jnp.ones((1, 128), f32), jnp.zeros((DP - DH - 1, 128), f32)], axis=0)

    def proj_v(t):
        def f():
            v = jnp.dot(wT[2 * D:, :], ln1_s[:, ts(t)], preferred_element_type=f32)
            for h in range(H):
                vT_s[h, :, ts(t)] = jnp.concatenate([v[h * DH:(h + 1) * DH], vtail], axis=0).astype(bf16)
        return f

    def wo_prep_pieces():
        ps = []
        def a():
            wt_f[0:D, :] = wo_v[...].astype(f32)
        ps.append(a)
        for g in range(4):
            def b(g=g):
                for h in range(4 * g, 4 * g + 4):
                    wt_f[D + h * DP: D + (h + 1) * DP, :] = jnp.concatenate([wt_f[h * DH:(h + 1) * DH, :], zpad], axis=0)
                woTp[:, g * 128:(g + 1) * 128] = wt_f[D + g * 128: D + (g + 1) * 128, :].T.astype(bf16)
            ps.append(b)
        return ps

    cp_x0.wait()
    cp_x1.start()
    cp_x23.start()
    cp_wkv.start()
    for t in range(4):
        ln1(t)()
    cp_wq.wait()
    for c in range(4):
        wt_chunk(c)()
    for t in range(0, 3):
        proj_q(t)()
    cp_x1.wait()
    for t in range(3, 7):
        proj_q(t)()
        ln1(t + 1)()
    cp_x23.wait()
    for t in range(7, 12):
        proj_q(t)()
        ln1(t + 1)()
    cp_wkv.wait()
    cp_wo.start()
    cp1.start()
    cp2.start()
    bk = [wt_chunk(c) for c in range(4, 7)]
    bv = [wt_chunk(c) for c in range(7, 11)]
    for i, t in enumerate(range(12, 16)):
        proj_q(t)()
        if t + 1 <= 15:
            ln1(t + 1)()
        for f in bk[i: i + 1]:
            f()
    for t in range(NT):
        proj_k(t)()
        if t % 2 == 0 and t // 2 < len(bv):
            bv[t // 2]()
    for t in range(NT):
        proj_v(t)()

    def hrows(h):
        if isinstance(h, int):
            return slice(h * DP, (h + 1) * DP)
        return pl.ds(pl.multiple_of(h * DP, DP), DP)

    def head(uq):
        qb, hf, k = uq
        return hf * (H // 2) + k

    def qk_chunk(uq, c, s_ref, mrun):
        qb, hf, k = uq
        s = jnp.dot(k_s[head(uq), c * CK:(c + 1) * CK, :], qT_s[qb, hf, k * DH:(k + 1) * DH, :],
                    preferred_element_type=f32)
        s_ref[c * CK:(c + 1) * CK, :] = s
        mc = jnp.max(s.reshape(CK // 8, 8, QB), axis=0)
        return mc if mrun is None else jnp.maximum(mrun, mc)

    def pv_chunk(uq, c, s_ref, m, acc):
        p = jnp.exp2(s_ref[c * CK:(c + 1) * CK, :] - m).astype(bf16)
        o = jnp.dot(vT_s[head(uq), :, c * CK:(c + 1) * CK], p, preferred_element_type=f32)
        return o if acc is None else acc + o

    def finalize(uq, acc):
        l = acc[DH:DH + 1, :]
        oT_s[uq[0], hrows(head(uq)), :] = (acc * pl.reciprocal(l, approx=False)).astype(bf16)

    def step(u_cur, u_next, s_cur, m_cur, s_next, m_next, fill=None):
        m = m_cur[...]
        mrun = None
        acc = None
        for t in range(NC + LAG):
            if fill is not None and t in fill:
                fill[t]()
            if t < NC and u_next is not None:
                mrun = qk_chunk(u_next, t, s_next, mrun)
            if t >= LAG:
                acc = pv_chunk(u_cur, t - LAG, s_cur, m, acc)
        if u_next is not None:
            m_next[...] = jnp.max(mrun, axis=0, keepdims=True)
        finalize(u_cur, acc)

    bufs = [(sA, sA, mA), (sB_ld, sB_st, mB)]

    mrun = None
    for c in range(NC):
        mrun = qk_chunk((0, 0, 0), c, sA, mrun)
    mA[...] = jnp.max(mrun, axis=0, keepdims=True)

    def units(base_units, nxt_last, fills=None):
        n = len(base_units)
        for k in range(n):
            cur = bufs[k % 2]; nx = bufs[(k + 1) % 2]
            u_next = base_units[k + 1] if k + 1 < n else nxt_last
            step(base_units[k], u_next, cur[0], cur[2], nx[1], nx[2], None if fills is None else fills[k])

    assert UPI == 8

    def body(i, carry):
        qb, hf = jax.lax.shift_right_logical(i, 1), i & 1
        qn, hn = jax.lax.shift_right_logical(i + 1, 1), (i + 1) & 1
        units([(qb, hf, k) for k in range(UPI)], (qn, hn, 0))
        return carry
    NIT = NU // UPI - 1
    jax.lax.fori_loop(0, NIT, body, 0)
    cp1.wait()
    cp2.wait()
    cp_wo.wait()

    def c_piece(t):
        def f():
            a = jnp.dot(woTp[...], oT_s[t // 4, :, ts(t % 4)], preferred_element_type=f32)
            hT = xT_v[:, ts(t)].astype(f32) + a
            hT_s[:, ts(t)] = hT
            mu, r = ln_stats(hT)
            ln_apply(hT_s, t, ln2T_s, mu, r)
        return f

    b1 = b1_ref[...].astype(f32)
    b2 = b2_ref[...].astype(f32)
    uacc = {}

    def d1_piece(c, k0, k1):
        def f():
            ks = slice(k0 * 128, k1 * 128)
            p = jnp.dot(ln2T_s[:, ks], w1_v[ks, c * FC:(c + 1) * FC], preferred_element_type=f32)
            uacc[c] = p if c not in uacc else uacc[c] + p
        return f

    def d1_finish(c, u):
        n = FC // 128
        bias = jnp.concatenate([b1[c * n + t: c * n + t + 1, :] for t in range(n)], axis=1)
        g_s[:, c * FC:(c + 1) * FC] = _gelu(u + bias).astype(bf16)

    cq = [c_piece(t) for t in range(12)]
    fills = [dict() for _ in range(UPI)]
    for f, t in zip(wo_prep_pieces(), (1, 3, 6, 9, 12)):
        fills[0][t] = f
    slots = [(k, t) for k in range(1, UPI - 1) for t in (4, 12)]
    for f, (k, t) in zip(cq, slots):
        fills[k][t] = f
    assert len(cq) <= len(slots)
    fills[UPI - 1] = {0: d1_piece(0, 0, 2), 3: d1_piece(0, 2, 4), 6: d1_piece(0, 4, 6), 9: d1_piece(0, 6, 8),
                      12: d1_piece(0, 8, 10), 15: d1_piece(0, 10, 12)}
    units([(NQB - 1, 1, k) for k in range(UPI)], None, fills)
    d1_piece(1, 0, 4)()
    c_piece(12)()
    c_piece(13)()
    d1_piece(1, 4, 8)()
    c_piece(14)()
    c_piece(15)()
    d1_piece(1, 8, 12)()
    d1_piece(0, 12, 16)()
    d1_finish(0, uacc[0])
    d1_piece(1, 12, 16)()
    d1_finish(1, uacc[1])
    for c in range(2, F // FC):
        u = jnp.dot(ln2T_s[...], w1_v[:, c * FC:(c + 1) * FC], preferred_element_type=f32)
        d1_finish(c, u)
    cps = []
    bounds = [0, 256, 512, 768, 1024, 1280, 1536, 1792, 1920, 2048]
    for c in range(len(bounds) - 1):
        lo, hi = bounds[c], bounds[c + 1]
        cs = slice(lo, hi)
        y = jnp.dot(g_s[...], w2_v[:, cs], preferred_element_type=f32)
        bias = jnp.concatenate([b2[t: t + 1, :] for t in range(lo // 128, hi // 128)], axis=1)
        out_v[:, cs] = (y + bias + hT_s[:, cs]).astype(bf16)
        cp = pltpu.make_async_copy(out_v.at[:, cs], out_hbm.at[:, cs], sems.at[8 + c])
        cp.start()
        cps.append(cp)
    for cp in cps:
        cp.wait()


@jax.jit
def pallas_sequential_preLN__mha_block__mixer_token_mlp__prompt_kernel(A_x, A_wqkv, A_wo, B_x, B_w1, B_b1, B_w2, B_b2):
    xT = A_x.reshape(S, D).T
    b1 = B_b1.reshape(F // 128, 128)
    b2 = B_b2.reshape(S // 128, 128)
    vm = pl.BlockSpec(memory_space=pltpu.VMEM)
    hbm = pl.BlockSpec(memory_space=pl.ANY)
    outT = pl.pallas_call(
        kernel,
        out_shape=jax.ShapeDtypeStruct((D, S), bf16),
        in_specs=[hbm, hbm, hbm, vm, vm, hbm, hbm],
        out_specs=hbm,
        scratch_shapes=[
            pltpu.SMEM((2,), jnp.int32),
            pltpu.SemaphoreType.DMA((20,)),
            pltpu.VMEM((D, S), bf16),
            pltpu.VMEM((D, 3 * D), bf16),
            pltpu.VMEM((D, D), bf16),
            pltpu.VMEM((S, F), bf16), pltpu.VMEM((F, S), bf16),
            pltpu.VMEM((D + DPAD, D), f32),
            pltpu.VMEM((3 * D, D), bf16),
            pltpu.VMEM((D, DPAD), bf16),
            pltpu.VMEM((D, S), bf16),
            pltpu.VMEM((H, S, DH), bf16),
            pltpu.VMEM((NQB, 2, HD, QB), bf16),
            pltpu.VMEM((H, DP, S), bf16),
            pltpu.VMEM((NQB, DPAD, QB), bf16),
            pltpu.VMEM((S, QB), f32), pltpu.VMEM((1, S, QB), f32),
            pltpu.VMEM((1, QB), f32), pltpu.VMEM((1, QB), f32),
            pltpu.VMEM((D, S), f32),
            pltpu.VMEM((D, S), bf16),
            pltpu.VMEM((D, F), bf16),
            pltpu.VMEM((D, S), bf16),
        ],
        compiler_params=pltpu.CompilerParams(vmem_limit_bytes=120 * 1024 * 1024),
    )(xT, A_wqkv, A_wo, b1, b2, B_w1, B_w2)
    return outT.T.reshape(1, S, D)
```

```python
import math

import jax
import jax.numpy as jnp
from jax.experimental import pallas as pl
from jax.experimental.pallas import tpu as pltpu

S, D, H, DH, DP, F = 2048, 448, 16, 28, 32, 1792
DPAD = H * DP
HD = D // 2
QB = 512
NQB = S // QB
NU = H * NQB
NT = S // 128
CK = 128
NC = S // CK
UPI = 8
LAG = 2
FC = 256
f32, bf16 = jnp.float32, jnp.bfloat16
QSCALE = (DH ** -0.5) * math.log2(math.e)
EPS = 1e-5


def _gelu(x):
    c = math.sqrt(2.0 / math.pi)
    return 0.5 * x * (1.0 + jnp.tanh(c * (x + 0.044715 * (x * x * x))))


def _colsum(x):
    n = x.shape[1]
    y = jnp.sum(x.reshape(8, 56, n), axis=0)
    y = jnp.sum(y.reshape(7, 8, n), axis=0)
    return jnp.sum(y, axis=0, keepdims=True)


def _kernel(xT_hbm, wqkv_hbm, wo_hbm, b1_ref, b2_ref, w1_hbm, w2_hbm, out_hbm,
            z_ref, sems, xT_v, wqkv_v, wo_v, w1_v, w2_v, wt_f, wT, woTp, ln1_s,
            k_s, qT_s, vT_s, oT_s, sA, sB, mA, mB, hT_s, ln2T_s, g_s, out_v):
    def xcopy(lo, hi, sem):
        return pltpu.make_async_copy(xT_hbm.at[:, lo:hi], xT_v.at[:, lo:hi], sems.at[sem])

    WQ = 512
    cp_x0 = xcopy(0, QB, 0)
    cp_wq = pltpu.make_async_copy(wqkv_hbm.at[:, 0:WQ], wqkv_v.at[:, 0:WQ], sems.at[1])
    cp_x1 = xcopy(QB, 2 * QB, 2)
    cp_x23 = xcopy(2 * QB, S, 3)
    cp_wkv = pltpu.make_async_copy(wqkv_hbm.at[:, WQ:], wqkv_v.at[:, WQ:], sems.at[4])
    cp_wo = pltpu.make_async_copy(wo_hbm, wo_v, sems.at[5])
    cp_w1 = pltpu.make_async_copy(w1_hbm, w1_v, sems.at[6])
    cp_w2 = pltpu.make_async_copy(w2_hbm, w2_v, sems.at[7])
    cp_x0.start()
    cp_wq.start()

    def ts(t):
        return slice(t * 128, (t + 1) * 128)

    z_ref[0] = 0
    z_ref[1] = 0
    sB_st = sB.at[z_ref[0]]
    sB_ld = sB.at[z_ref[1]]
    rows_dyn = pl.ds(pl.multiple_of(z_ref[1], 16), D)

    def ln_stats(x, twice=False):
        p = x[0:1, :]
        d = x - p
        md = _colsum(d) * (1.0 / D)
        var = jnp.maximum(_colsum(d * d) * (1.0 / D) - md * md, 0.0)
        r = jax.lax.rsqrt(var + EPS)
        if twice:
            r = r * jax.lax.rsqrt(var * r * r + EPS)
        return p + md, r

    def ln_apply(src_ref, t, dst_ref, mu, r):
        dst_ref[:, ts(t)] = ((src_ref[rows_dyn, ts(t)].astype(f32) - mu) * r).astype(bf16)

    def wt_chunk(c):
        lo = c * 128
        hi = min(lo + 128, 3 * D)
        wT[lo:hi, :] = wqkv_v[:, lo:hi].astype(f32).T.astype(bf16)

    def ln1(t):
        mu, r = ln_stats(xT_v[:, ts(t)].astype(f32))
        ln_apply(xT_v, t, ln1_s, mu, r)

    def proj_q(t):
        q = jnp.dot(wT[0:D, :], ln1_s[:, ts(t)], preferred_element_type=f32)
        q = (q * QSCALE).astype(bf16)
        qT_s[t // 4, 0, :, ts(t % 4)] = q[0:HD]
        qT_s[t // 4, 1, :, ts(t % 4)] = q[HD:]

    def proj_k(t):
        kT = jnp.dot(wT[D:2 * D, :], ln1_s[:, ts(t)], preferred_element_type=f32)
        k = kT.T.astype(bf16)
        for h in range(H):
            k_s[h, ts(t), :] = k[:, h * DH:(h + 1) * DH]

    vtail = jnp.concatenate([jnp.ones((1, 128), f32), jnp.zeros((DP - DH - 1, 128), f32)], axis=0)

    def proj_v(t):
        v = jnp.dot(wT[2 * D:, :], ln1_s[:, ts(t)], preferred_element_type=f32)
        for h in range(H):
            vT_s[h, :, ts(t)] = jnp.concatenate([v[h * DH:(h + 1) * DH], vtail], axis=0).astype(bf16)

    def wo_prep_pieces():
        zpad = jnp.zeros((DP - DH, D), f32)

        def first():
            wt_f[0:D, :] = wo_v[...].astype(f32)

        def group(g):
            def f():
                for h in range(4 * g, 4 * g + 4):
                    wt_f[D + h * DP: D + (h + 1) * DP, :] = jnp.concatenate(
                        [wt_f[h * DH:(h + 1) * DH, :], zpad], axis=0)
                woTp[:, g * 128:(g + 1) * 128] = wt_f[D + g * 128: D + (g + 1) * 128, :].T.astype(bf16)
            return f
        return [first] + [group(g) for g in range(4)]

    cp_x0.wait()
    cp_x1.start()
    cp_x23.start()
    cp_wkv.start()
    for t in range(4):
        ln1(t)
    cp_wq.wait()
    for c in range(4):
        wt_chunk(c)
    for t in range(0, 3):
        proj_q(t)
    cp_x1.wait()
    for t in range(3, 7):
        proj_q(t)
        ln1(t + 1)
    cp_x23.wait()
    for t in range(7, 12):
        proj_q(t)
        ln1(t + 1)
    cp_wkv.wait()
    cp_wo.start()
    cp_w1.start()
    cp_w2.start()
    for i, t in enumerate(range(12, 16)):
        proj_q(t)
        if t + 1 < NT:
            ln1(t + 1)
        if i < 3:
            wt_chunk(4 + i)
    for t in range(NT):
        proj_k(t)
        if t % 2 == 0 and t // 2 < 4:
            wt_chunk(7 + t // 2)
    for t in range(NT):
        proj_v(t)

    def head(uq):
        return uq[1] * (H // 2) + uq[2]

    def hrows(h):
        if isinstance(h, int):
            return slice(h * DP, (h + 1) * DP)
        return pl.ds(pl.multiple_of(h * DP, DP), DP)

    def qk_chunk(uq, c, s_ref, mrun):
        qb, hf, k = uq
        s = jnp.dot(k_s[head(uq), c * CK:(c + 1) * CK, :], qT_s[qb, hf, k * DH:(k + 1) * DH, :],
                    preferred_element_type=f32)
        s_ref[c * CK:(c + 1) * CK, :] = s
        mc = jnp.max(s.reshape(CK // 8, 8, QB), axis=0)
        return mc if mrun is None else jnp.maximum(mrun, mc)

    def pv_chunk(uq, c, s_ref, m, acc):
        p = jnp.exp2(s_ref[c * CK:(c + 1) * CK, :] - m).astype(bf16)
        o = jnp.dot(vT_s[head(uq), :, c * CK:(c + 1) * CK], p, preferred_element_type=f32)
        return o if acc is None else acc + o

    def finalize(uq, acc):
        l = acc[DH:DH + 1, :]
        oT_s[uq[0], hrows(head(uq)), :] = (acc * pl.reciprocal(l, approx=False)).astype(bf16)

    def step(u_cur, u_next, s_cur, m_cur, s_next, m_next, fill=None):
        m = m_cur[...]
        mrun = None
        acc = None
        for t in range(NC + LAG):
            if fill is not None and t in fill:
                fill[t]()
            if t < NC and u_next is not None:
                mrun = qk_chunk(u_next, t, s_next, mrun)
            if t >= LAG:
                acc = pv_chunk(u_cur, t - LAG, s_cur, m, acc)
        if u_next is not None:
            m_next[...] = jnp.max(mrun, axis=0, keepdims=True)
        finalize(u_cur, acc)

    bufs = [(sA, sA, mA), (sB_ld, sB_st, mB)]

    mrun = None
    for c in range(NC):
        mrun = qk_chunk((0, 0, 0), c, sA, mrun)
    mA[...] = jnp.max(mrun, axis=0, keepdims=True)

    def units(base_units, nxt_last, fills=None):
        n = len(base_units)
        for k in range(n):
            cur, nx = bufs[k % 2], bufs[(k + 1) % 2]
            u_next = base_units[k + 1] if k + 1 < n else nxt_last
            step(base_units[k], u_next, cur[0], cur[2], nx[1], nx[2], None if fills is None else fills[k])

    def body(i, carry):
        qb, hf = jax.lax.shift_right_logical(i, 1), i & 1
        qn, hn = jax.lax.shift_right_logical(i + 1, 1), (i + 1) & 1
        units([(qb, hf, k) for k in range(UPI)], (qn, hn, 0))
        return carry

    jax.lax.fori_loop(0, NU // UPI - 1, body, 0)
    cp_w1.wait()
    cp_w2.wait()
    cp_wo.wait()

    def c_piece(t):
        def f():
            a = jnp.dot(woTp[...], oT_s[t // 4, :, ts(t % 4)], preferred_element_type=f32)
            hT = xT_v[:, ts(t)].astype(f32) + a
            hT_s[:, ts(t)] = hT
            mu, r = ln_stats(hT, twice=True)
            ln_apply(hT_s, t, ln2T_s, mu, r)
        return f

    b1 = b1_ref[...].astype(f32)
    b2 = b2_ref[...].astype(f32)
    uacc = {}

    def d1_piece(c, k0, k1):
        def f():
            ks = slice(k0 * 128, k1 * 128)
            p = jnp.dot(ln2T_s[:, ks], w1_v[ks, c * FC:(c + 1) * FC], preferred_element_type=f32)
            uacc[c] = p if c not in uacc else uacc[c] + p
        return f

    def d1_finish(c, u):
        n = FC // 128
        bias = jnp.concatenate([b1[c * n + t: c * n + t + 1, :] for t in range(n)], axis=1)
        g_s[:, c * FC:(c + 1) * FC] = _gelu(u + bias).astype(bf16)

    fills = [dict() for _ in range(UPI)]
    for f, t in zip(wo_prep_pieces(), (1, 3, 6, 9, 12)):
        fills[0][t] = f
    slots = [(k, t) for k in range(1, UPI - 1) for t in (4, 12)]
    for f, (k, t) in zip([c_piece(t) for t in range(12)], slots):
        fills[k][t] = f
    fills[UPI - 1] = {0: d1_piece(0, 0, 2), 3: d1_piece(0, 2, 4), 6: d1_piece(0, 4, 6), 9: d1_piece(0, 6, 8),
                      12: d1_piece(0, 8, 10), 15: d1_piece(0, 10, 12)}
    units([(NQB - 1, 1, k) for k in range(UPI)], None, fills)
    d1_piece(1, 0, 4)()
    c_piece(12)()
    c_piece(13)()
    d1_piece(1, 4, 8)()
    c_piece(14)()
    c_piece(15)()
    d1_piece(1, 8, 12)()
    d1_piece(0, 12, 16)()
    d1_finish(0, uacc[0])
    d1_piece(1, 12, 16)()
    d1_finish(1, uacc[1])
    for c in range(2, F // FC):
        u = jnp.dot(ln2T_s[...], w1_v[:, c * FC:(c + 1) * FC], preferred_element_type=f32)
        d1_finish(c, u)

    out_copies = []
    bounds = [0, 256, 512, 768, 1024, 1280, 1536, 1792, 1920, 2048]
    for c in range(len(bounds) - 1):
        lo, hi = bounds[c], bounds[c + 1]
        cs = slice(lo, hi)
        y = jnp.dot(g_s[...], w2_v[:, cs], preferred_element_type=f32)
        bias = jnp.concatenate([b2[t: t + 1, :] for t in range(lo // 128, hi // 128)], axis=1)
        out_v[:, cs] = (y + bias + hT_s[:, cs]).astype(bf16)
        cp = pltpu.make_async_copy(out_v.at[:, cs], out_hbm.at[:, cs], sems.at[8 + c])
        cp.start()
        out_copies.append(cp)
    for cp in out_copies:
        cp.wait()


@jax.jit
def pallas_sequential_preLN__mha_block__mixer_token_mlp__prompt_kernel(
        A_x, A_wqkv, A_wo, B_x, B_w1, B_b1, B_w2, B_b2):
    del B_x
    xT = A_x.reshape(S, D).T
    b1 = B_b1.reshape(F // 128, 128)
    b2 = B_b2.reshape(S // 128, 128)
    vm = pl.BlockSpec(memory_space=pltpu.VMEM)
    hbm = pl.BlockSpec(memory_space=pl.ANY)
    outT = pl.pallas_call(
        _kernel,
        out_shape=jax.ShapeDtypeStruct((D, S), bf16),
        in_specs=[hbm, hbm, hbm, vm, vm, hbm, hbm],
        out_specs=hbm,
        scratch_shapes=[
            pltpu.SMEM((2,), jnp.int32),
            pltpu.SemaphoreType.DMA((20,)),
            pltpu.VMEM((D, S), bf16),
            pltpu.VMEM((D, 3 * D), bf16),
            pltpu.VMEM((D, D), bf16),
            pltpu.VMEM((S, F), bf16),
            pltpu.VMEM((F, S), bf16),
            pltpu.VMEM((D + DPAD, D), f32),
            pltpu.VMEM((3 * D, D), bf16),
            pltpu.VMEM((D, DPAD), bf16),
            pltpu.VMEM((D, S), bf16),
            pltpu.VMEM((H, S, DH), bf16),
            pltpu.VMEM((NQB, 2, HD, QB), bf16),
            pltpu.VMEM((H, DP, S), bf16),
            pltpu.VMEM((NQB, DPAD, QB), bf16),
            pltpu.VMEM((S, QB), f32),
            pltpu.VMEM((1, S, QB), f32),
            pltpu.VMEM((1, QB), f32),
            pltpu.VMEM((1, QB), f32),
            pltpu.VMEM((D, S), f32),
            pltpu.VMEM((D, S), bf16),
            pltpu.VMEM((D, F), bf16),
            pltpu.VMEM((D, S), bf16),
        ],
        compiler_params=pltpu.CompilerParams(vmem_limit_bytes=120 * 1024 * 1024),
    )(xT, A_wqkv, A_wo, b1, b2, B_w1, B_w2)
    return outT.T.reshape(1, S, D)
```
